```python
import os as _os
_os.environ.setdefault("JAX_PLATFORMS", "cpu")
import jax
import jax.numpy as jnp

def _softmax(x, axis=-1):
    return jax.nn.softmax(x, axis=axis)
def _gelu(x):
    return jax.nn.gelu(x, approximate=True)
def _silu(x):
    return jax.nn.silu(x)
def _sigmoid(x):
    return jax.nn.sigmoid(x)
def _layernorm(x, axis=-1, eps=1e-5):
    m = jnp.mean(x, axis=axis, keepdims=True)
    v = jnp.var(x, axis=axis, keepdims=True)
    return (x - m) / jnp.sqrt(v + eps)
def _scatter_add(tgt, idx, src, axis=0):
    return tgt.at[idx].add(src)
def _segment_sum(src, seg, n):
    return jax.ops.segment_sum(src, seg, n)
class _Rng:
    def __init__(self, key):
        self._k = key
    def _next(self):
        self._k, sub = jax.random.split(self._k)
        return sub
    def normal(self, shape):
        return jax.random.normal(self._next(), shape, dtype=jnp.bfloat16)
    def randint(self, lo, hi, shape):
        return jax.random.randint(self._next(), shape, lo, hi, dtype=jnp.int32)
    def uniform(self, shape, lo=0.0, hi=1.0):
        return jax.random.uniform(self._next(), shape, jnp.bfloat16, lo, hi)
    def permutation(self, n):
        return jax.random.permutation(self._next(), n)


kernel_name = 'concat_heads__gqa_block_cached__gqa_block_cached__near_ridge'

def setup_inputs():
    _rng = _Rng(jax.random.key(int.from_bytes(__import__("os").urandom(4), "little")))
    _w = (lambda a: (lambda t: t.astype(jnp.bfloat16) if jnp.issubdtype(t.dtype, jnp.floating) else t)(jnp.asarray(a)))
    def _A_setup():
        B, Sq, D = 8, 128, 576
        Hq, Hkv, Sk, Dh = 32, 16, 512, 128
        assert Hq % Hkv == 0, (Hq, Hkv)
        return {
            "x": _w((lambda *s: _rng.normal(s) * 0.8)(B, Sq, D)),
            "k_cache": _w((lambda *s: _rng.normal(s) * 0.8)(B, Hkv, Sk, Dh)),
            "v_cache": _w((lambda *s: _rng.normal(s) * 0.05)(B, Hkv, Sk, Dh)),
            "wq": _w((lambda *s: _rng.normal(s) * 0.8)(D, Hq * Dh) * (D ** -0.5)),
            "wo": _w((lambda *s: _rng.normal(s) * 0.05)(Hq * Dh, D) * ((Hq * Dh) ** -0.5)),
        }
    _A_in = _A_setup()

    def _B_setup():
        B, Sq, D = 8, 128, 576
        Hq, Hkv, Sk, Dh = 32, 16, 512, 128
        assert Hq % Hkv == 0, (Hq, Hkv)
        return {
            "x": _w((lambda *s: _rng.normal(s) * 0.8)(B, Sq, D)),
            "k_cache": _w((lambda *s: _rng.normal(s) * 0.8)(B, Hkv, Sk, Dh)),
            "v_cache": _w((lambda *s: _rng.normal(s) * 0.05)(B, Hkv, Sk, Dh)),
            "wq": _w((lambda *s: _rng.normal(s) * 0.8)(D, Hq * Dh) * (D ** -0.5)),
            "wo": _w((lambda *s: _rng.normal(s) * 0.05)(Hq * Dh, D) * ((Hq * Dh) ** -0.5)),
        }
    _B_in = _B_setup()

    return {
        "A_x": _A_in["x"],
        "A_k_cache": _A_in["k_cache"],
        "A_v_cache": _A_in["v_cache"],
        "A_wq": _A_in["wq"],
        "A_wo": _A_in["wo"],
        "B_x": _B_in["x"],
        "B_k_cache": _B_in["k_cache"],
        "B_v_cache": _B_in["v_cache"],
        "B_wq": _B_in["wq"],
        "B_wo": _B_in["wo"],
    }

def reference(A_x, A_k_cache, A_v_cache, A_wq, A_wo, B_x, B_k_cache, B_v_cache, B_wq, B_wo):
    def _A_ref(x, k_cache, v_cache, wq, wo):
        B, Sq, D = x.shape
        Hq, Dh = 32, 128
        Hkv = k_cache.shape[1]
        rep = Hq // Hkv
        q = (lambda x, *d: x.transpose(*d))((x @ wq).reshape(B, Sq, Hq, Dh), 0, 2, 1, 3)
        k = jnp.repeat(k_cache, rep, axis=1)
        v = jnp.repeat(v_cache, rep, axis=1)
        scores = jnp.einsum("bhqd,bhkd->bhqk", q, k) * (Dh ** -0.5)
        p = _softmax(scores, axis=-1)
        o = jnp.einsum("bhqk,bhkd->bhqd", p, v)
        return (lambda x, *d: x.transpose(*d))(o, 0, 2, 1, 3).reshape(B, Sq, Hq * Dh) @ wo

    def _B_ref(x, k_cache, v_cache, wq, wo):
        B, Sq, D = x.shape
        Hq, Dh = 32, 128
        Hkv = k_cache.shape[1]
        rep = Hq // Hkv
        q = (lambda x, *d: x.transpose(*d))((x @ wq).reshape(B, Sq, Hq, Dh), 0, 2, 1, 3)
        k = jnp.repeat(k_cache, rep, axis=1)
        v = jnp.repeat(v_cache, rep, axis=1)
        scores = jnp.einsum("bhqd,bhkd->bhqk", q, k) * (Dh ** -0.5)
        p = _softmax(scores, axis=-1)
        o = jnp.einsum("bhqk,bhkd->bhqd", p, v)
        return (lambda x, *d: x.transpose(*d))(o, 0, 2, 1, 3).reshape(B, Sq, Hq * Dh) @ wo

    a = _A_ref(A_x, A_k_cache, A_v_cache, A_wq, A_wo)
    b = _B_ref(B_x, B_k_cache, B_v_cache, B_wq, B_wo)
    return jnp.concatenate([a, b], axis=-1)
```

```python
import jax
import jax.numpy as jnp
import numpy as np
import jax.experimental.pallas as pl
import jax.experimental.pallas.tpu as pltpu

B, Sq, D = 8, 128, 576
Hq, Hkv, Sk, Dh = 32, 16, 512, 128
HD = Hq * Dh
SCALE = float(Dh ** -0.5) * float(np.log2(np.e))
NU = 2 * B
F32 = jnp.float32
BF16 = jnp.bfloat16

SK = 4
NS = 4
PFD = 2
HH = Hkv // 2
LP = 1
WQCH = [512, 512, 1024, 1024, 1024]
WQOFF = [sum(WQCH[:c]) for c in range(len(WQCH))]
PW = 1024
ENDSPLIT = (3, 2)

S_X, S_WQB, S_WO, S_K = 0, 4, 5, 7
S_OUT = S_K + 3 * NS
S_WQ = S_OUT + B
S_END = S_WQ + len(WQCH)
NSEM = S_END + 6


def _kernel(xa, ka, va, wqa, woa, xb, kb, vb, wqb, wob, out_hbm,
            xt_v, x_v, wq_v, wo_v, k_v, v_v, q_v, o_v, outT_v, out_v, p_v, sems):

    def x_copy(j):
        if j < 3:
            lo, hi = ((0, 2), (2, 4), (4, 8))[j]
            return pltpu.make_async_copy(xa.at[lo:hi], xt_v.at[0, lo:hi], sems.at[S_X + j])
        return pltpu.make_async_copy(xb, xt_v.at[1], sems.at[S_X + 3])

    def wqa_copy(c):
        cols = pl.ds(WQOFF[c], WQCH[c])
        return pltpu.make_async_copy(wqa.at[:, cols], wq_v.at[0, :, cols], sems.at[S_WQ + c])

    def wqb_copy():
        return pltpu.make_async_copy(wqb, wq_v.at[1], sems.at[S_WQB])

    def wo_copy(br):
        return pltpu.make_async_copy((woa, wob)[br], wo_v.at[br], sems.at[S_WO + br])

    def kv_copy(u, part, for_wait=False):
        srcs, dst = ((ka, kb), k_v) if part == 0 else ((va, vb), v_v)
        hs = (pl.ds(0, Hkv), pl.ds(0, HH), pl.ds(HH, HH))[part]
        slot = u & (NS - 1)
        if isinstance(u, int):
            src = srcs[u // B].at[u % B, hs]
        elif for_wait:
            src = srcs[0].at[0, hs]
        else:
            b = u & (B - 1)
            src = pl.select_ref(u >> 3, srcs[0].at[b, hs], srcs[1].at[b, hs])
        return pltpu.make_async_copy(src, dst.at[slot, hs], sems.at[S_K + part * NS + slot])

    def kv_start(u):
        for part in range(3):
            kv_copy(u, part).start(priority=LP)

    def out_copy(u):
        return pltpu.make_async_copy(out_v.at[u & 7], out_hbm.at[u & 7], sems.at[S_OUT + (u & 7)])

    def when(cond, fn):
        if isinstance(cond, (bool, np.bool_)):
            if cond:
                fn()
        else:
            def _f():
                fn()
            pl.when(cond)(_f)

    def qproj(u):
        q = jnp.dot(x_v[u & 7], wq_v[u >> 3], preferred_element_type=F32)
        q_v[u & 7] = (q * SCALE).astype(BF16)

    def qk_part(u, h):
        q2 = jnp.concatenate([q_v[u & 7, :, pl.ds((2 * h) * Dh, Dh)],
                              q_v[u & 7, :, pl.ds((2 * h + 1) * Dh, Dh)]], axis=0)
        return jax.lax.dot_general(q2, k_v[u & (NS - 1), h], (((1,), (1,)), ((), ())),
                                   preferred_element_type=F32)

    def sm_part(s, h):
        m = jnp.max(s, axis=-1, keepdims=True)
        p = jnp.exp2(s - m)
        l = jnp.sum(p, axis=-1, keepdims=True)
        p_v[h & 1] = p.astype(BF16)
        return pltpu.reciprocal(l, approx=True)

    def pv_part(u, h, r):
        o = jnp.dot(p_v[h & 1], v_v[u & (NS - 1), h], preferred_element_type=F32)
        o = (o * r).astype(BF16)
        o_v[u & 1, :, pl.ds((2 * h) * Dh, Dh)] = o[:Sq]
        o_v[u & 1, :, pl.ds((2 * h + 1) * Dh, Dh)] = o[Sq:]

    def attention(i, hooks):
        s_cur = qk_part(i, 0)
        for h in range(Hkv):
            s_nxt = qk_part(i, h + 1) if h + 1 < Hkv else None
            r = sm_part(s_cur, h)
            if h in hooks:
                hooks[h]()
            pv_part(i, h, r)
            s_cur = s_nxt

    def oproj_val(u):
        return jax.lax.dot_general(wo_v[u >> 3], o_v[u & 1], (((1,), (1,)), ((), ())),
                                   preferred_element_type=F32).astype(BF16)

    def finish(u):
        off = (u >> 3) * 512 if isinstance(u, int) else pl.multiple_of((u >> 3) * 512, 512)
        out_v[u & 7, :, pl.ds(off, 640)] = outT_v[u & 7, pl.ds(off, 640), :].T

    def fin_direct(u):
        b = u & 7
        full = jnp.concatenate([outT_v[b, pl.ds(512, 64), :], oproj_val(u)], axis=0)
        out_v[b, :, pl.ds(512, 640)] = full.T

    def dma_top(i):
        kv_copy(i, 0, True).wait()
        kv_copy(i, 1, True).wait()

    def dma_starts(i, do_q, outs):
        for u in outs:
            when(u >= B, lambda: out_copy(u).start())
        nxt = i + PFD
        when(nxt < NU, lambda: kv_start(nxt))
        if do_q:
            when(i == 1, lambda: (x_copy(3).start(priority=LP), wqb_copy().start(priority=LP)))
            when(i == 4, lambda: wo_copy(1).start(priority=LP))

    def dma_mid(i, outs):
        dma_starts(i, False, outs)
        kv_copy(i, 2, True).wait()

    def unit_main(i):
        dma_top(i)
        kv_copy(i, 2, True).wait()
        when(i + SK == B, lambda: x_copy(3).wait())
        x_v[(i + SK) & 7] = xt_v[(i + SK) >> 3, (i + SK) & 7].T
        finish(jnp.maximum(i - 1, 0))

        def qh():
            when(i + SK == B, lambda: wqb_copy().wait())
            qproj(i + SK)
        attention(i, {Hkv - 1: qh})
        dma_starts(i, True, (i - 2,))
        when((i & 7) == 0,
             lambda: pltpu.make_async_copy(woa, wo_v.at[i >> 3], sems.at[S_WO + (i >> 3)]).wait())
        outT_v[i & 7, pl.ds(pl.multiple_of((i >> 3) * D, 64), D), :] = oproj_val(i)

    x_copy(0).start(priority=0)
    wqa_copy(0).start(priority=LP)
    x_copy(1).start(priority=LP)
    for c in range(1, len(WQCH)):
        wqa_copy(c).start(priority=LP)
    outT_v[:, pl.ds(D, 64), :] = jnp.zeros((B, 64, Sq), BF16)
    outT_v[0, pl.ds(0, D), :] = jnp.zeros((D, Sq), BF16)

    def pchunk(u0, nu, cols):
        x0 = jnp.concatenate([x_v[u] for u in range(u0, u0 + nu)], axis=0)
        q = (jnp.dot(x0, wq_v[0, :, cols], preferred_element_type=F32) * SCALE).astype(BF16)
        for t in range(nu):
            q_v[u0 + t, :, cols] = q[t * Sq:(t + 1) * Sq]

    x_copy(0).wait()
    x_v[0] = xt_v[0, 0].T
    x_v[1] = xt_v[0, 1].T
    wqa_copy(0).wait()
    pchunk(0, 2, pl.ds(WQOFF[0], WQCH[0]))
    x_copy(1).wait()
    x_v[2] = xt_v[0, 2].T
    x_v[3] = xt_v[0, 3].T
    pchunk(2, 2, pl.ds(WQOFF[0], WQCH[0]))
    x_copy(2).start(priority=LP)
    kv_start(0)
    wqa_copy(1).wait()
    pchunk(0, SK, pl.ds(WQOFF[1], WQCH[1]))
    wo_copy(0).start(priority=LP)
    kv_start(1)

    def pbody(c, _):
        pltpu.make_async_copy(wqa.at[:, pl.ds(1024, PW)], wq_v.at[0, :, pl.ds(1024, PW)],
                              sems.at[S_WQ + 2 + c]).wait()
        pchunk(0, SK, pl.ds(pl.multiple_of(1024 + c * PW, 512), PW))
        return 0
    jax.lax.fori_loop(0, 3072 // PW, pbody, 0)
    x_copy(2).wait()

    def main(b, _):
        unit_main(2 * b)
        unit_main(2 * b + 1)
        return 0
    jax.lax.fori_loop(0, (NU - SK) // 2, main, 0)

    T0 = NU - SK
    dma_top(T0)
    finish(T0 - 1)
    attention(T0, {HH: lambda: dma_mid(T0, (T0 - 2, T0 - 1))})

    def tail(i, _):
        dma_top(i)
        fin_direct(i - 1)
        attention(i, {HH: lambda: dma_mid(i, (i - 1,))})
        return 0
    jax.lax.fori_loop(T0 + 1, NU, tail, 0)

    b = B - 1

    def part(lo, hi, k):
        cols = pl.ds(lo, hi - lo)
        return pltpu.make_async_copy(out_v.at[b, :, cols], out_hbm.at[b, :, cols], sems.at[S_END + k])
    parts = [part(0, 512, 0)]
    parts[0].start()
    r0 = 0
    for k, nt in enumerate(ENDSPLIT):
        nr = 128 * nt - (64 if k == 0 else 0)
        r = jax.lax.dot_general(wo_v[1, pl.ds(r0, nr), :], o_v[(NU - 1) & 1], (((1,), (1,)), ((), ())),
                                preferred_element_type=F32).astype(BF16)
        if k == 0:
            r = jnp.concatenate([outT_v[b, pl.ds(512, 64), :], r], axis=0)
        lo = 512 if k == 0 else D + r0
        out_v[b, :, pl.ds(lo, 128 * nt)] = r.T
        parts.append(part(lo, lo + 128 * nt, k + 1))
        parts[-1].start()
        r0 += nr
    for u in range(B, NU - 1):
        out_copy(u).wait()
    for p in parts:
        p.wait()


@jax.jit
def pallas_concat_heads__gqa_block_cached__gqa_block_cached__near_ridge_kernel(
    A_x: jax.Array,
    A_k_cache: jax.Array,
    A_v_cache: jax.Array,
    A_wq: jax.Array,
    A_wo: jax.Array,
    B_x: jax.Array,
    B_k_cache: jax.Array,
    B_v_cache: jax.Array,
    B_wq: jax.Array,
    B_wo: jax.Array,
):
    hbm = pl.BlockSpec(memory_space=pltpu.HBM)
    return pl.pallas_call(
        _kernel,
        grid=(),
        in_specs=[hbm] * 10,
        out_specs=hbm,
        out_shape=jax.ShapeDtypeStruct((B, Sq, 2 * D), BF16),
        scratch_shapes=[
            pltpu.VMEM((2, B, D, Sq), BF16),
            pltpu.VMEM((8, Sq, D), BF16),
            pltpu.VMEM((2, D, HD), BF16),
            pltpu.VMEM((2, D, HD), BF16),
            pltpu.VMEM((NS, Hkv, Sk, Dh), BF16),
            pltpu.VMEM((NS, Hkv, Sk, Dh), BF16),
            pltpu.VMEM((8, Sq, HD), BF16),
            pltpu.VMEM((2, Sq, HD), BF16),
            pltpu.VMEM((B, 2 * D, Sq), BF16),
            pltpu.VMEM((B, Sq, 2 * D), BF16),
            pltpu.VMEM((2, 2 * Sq, Sk), BF16),
            pltpu.SemaphoreType.DMA((NSEM,)),
        ],
        compiler_params=pltpu.CompilerParams(
            vmem_limit_bytes=110 * 1024 * 1024,
            flags={"XLA_TPU_RESCHEDULE_DMA_DONES": True},
        ),
    )(A_x.transpose(0, 2, 1), A_k_cache, A_v_cache, A_wq, A_wo.T,
      B_x.transpose(0, 2, 1), B_k_cache, B_v_cache, B_wq, B_wo.T)
```

```python
import jax
import jax.numpy as jnp
import numpy as np
import jax.experimental.pallas as pl
import jax.experimental.pallas.tpu as pltpu

B, Sq, D = 8, 128, 576
Hq, Hkv, Sk, Dh = 32, 16, 512, 128
HD = Hq * Dh
SCALE = float(Dh ** -0.5) * float(np.log2(np.e))
NU = 2 * B
F32 = jnp.float32
BF16 = jnp.bfloat16

SK = 4
NS = 4
PFD = 2
HH = Hkv // 2
LP = 1
WQCH = [512, 512, 1024, 1024, 1024]
WQOFF = [sum(WQCH[:c]) for c in range(len(WQCH))]
PW = 1024
ENDSPLIT = (3, 2)

S_X, S_WQB, S_WO, S_K = 0, 4, 5, 7
S_OUT = S_K + 3 * NS
S_WQ = S_OUT + B
S_END = S_WQ + len(WQCH)
NSEM = S_END + 6


def _kernel(xa, ka, va, wqa, woa, xb, kb, vb, wqb, wob, out_hbm,
            xt_v, x_v, wq_v, wo_v, k_v, v_v, q_v, o_v, outT_v, out_v, p_v, sems):

    def x_copy(j):
        if j < 3:
            lo, hi = ((0, 2), (2, 4), (4, 8))[j]
            return pltpu.make_async_copy(xa.at[lo:hi], xt_v.at[0, lo:hi], sems.at[S_X + j])
        return pltpu.make_async_copy(xb, xt_v.at[1], sems.at[S_X + 3])

    def wqa_copy(c):
        cols = pl.ds(WQOFF[c], WQCH[c])
        return pltpu.make_async_copy(wqa.at[:, cols], wq_v.at[0, :, cols], sems.at[S_WQ + c])

    def wqb_copy():
        return pltpu.make_async_copy(wqb, wq_v.at[1], sems.at[S_WQB])

    def wo_copy(br):
        return pltpu.make_async_copy((woa, wob)[br], wo_v.at[br], sems.at[S_WO + br])

    def kv_copy(u, part, br=None):
        srcs, dst = ((ka, kb), k_v) if part == 0 else ((va, vb), v_v)
        hs = (pl.ds(0, Hkv), pl.ds(0, HH), pl.ds(HH, HH))[part]
        slot = u & (NS - 1)
        if isinstance(u, int):
            src = srcs[u // B].at[u % B, hs]
        elif br is None:
            src = srcs[0].at[0, hs]
        else:
            src = srcs[br].at[u & (B - 1), hs]
        return pltpu.make_async_copy(src, dst.at[slot, hs], sems.at[S_K + part * NS + slot])

    def kv_start(u):
        if isinstance(u, int):
            for part in range(3):
                kv_copy(u, part).start(priority=LP)
            return
        for br in range(2):
            @pl.when((u >> 3) == br)
            def _():
                for part in range(3):
                    kv_copy(u, part, br).start(priority=LP)

    def out_copy(u):
        return pltpu.make_async_copy(out_v.at[u & 7], out_hbm.at[u & 7], sems.at[S_OUT + (u & 7)])

    def when(cond, fn):
        if isinstance(cond, (bool, np.bool_)):
            if cond:
                fn()
        else:
            def _f():
                fn()
            pl.when(cond)(_f)

    def qproj(u):
        q = jnp.dot(x_v[u & 7], wq_v[u >> 3], preferred_element_type=F32)
        q_v[u & 7] = (q * SCALE).astype(BF16)

    def qk_part(u, h):
        q2 = jnp.concatenate([q_v[u & 7, :, pl.ds((2 * h) * Dh, Dh)],
                              q_v[u & 7, :, pl.ds((2 * h + 1) * Dh, Dh)]], axis=0)
        return jax.lax.dot_general(q2, k_v[u & (NS - 1), h], (((1,), (1,)), ((), ())),
                                   preferred_element_type=F32)

    def sm_part(s, h):
        m = jnp.max(s, axis=-1, keepdims=True)
        p = jnp.exp2(s - m)
        l = jnp.sum(p, axis=-1, keepdims=True)
        p_v[h & 1] = p.astype(BF16)
        return pltpu.reciprocal(l, approx=True)

    def pv_part(u, h, r):
        o = jnp.dot(p_v[h & 1], v_v[u & (NS - 1), h], preferred_element_type=F32)
        o = (o * r).astype(BF16)
        o_v[u & 1, :, pl.ds((2 * h) * Dh, Dh)] = o[:Sq]
        o_v[u & 1, :, pl.ds((2 * h + 1) * Dh, Dh)] = o[Sq:]

    def attention(i, hooks):
        s_cur = qk_part(i, 0)
        for h in range(Hkv):
            s_nxt = qk_part(i, h + 1) if h + 1 < Hkv else None
            r = sm_part(s_cur, h)
            if h in hooks:
                hooks[h]()
            pv_part(i, h, r)
            s_cur = s_nxt

    def oproj_val(u):
        return jax.lax.dot_general(wo_v[u >> 3], o_v[u & 1], (((1,), (1,)), ((), ())),
                                   preferred_element_type=F32).astype(BF16)

    def finish(u):
        off = (u >> 3) * 512 if isinstance(u, int) else pl.multiple_of((u >> 3) * 512, 512)
        out_v[u & 7, :, pl.ds(off, 640)] = outT_v[u & 7, pl.ds(off, 640), :].T

    def fin_direct(u):
        b = u & 7
        full = jnp.concatenate([outT_v[b, pl.ds(512, 64), :], oproj_val(u)], axis=0)
        out_v[b, :, pl.ds(512, 640)] = full.T

    def dma_top(i):
        kv_copy(i, 0).wait()
        kv_copy(i, 1).wait()

    def dma_starts(i, do_q, outs):
        for u in outs:
            when(u >= B, lambda: out_copy(u).start())
        nxt = i + PFD
        when(nxt < NU, lambda: kv_start(nxt))
        if do_q:
            when(i == 1, lambda: (x_copy(3).start(priority=LP), wqb_copy().start(priority=LP)))
            when(i == 4, lambda: wo_copy(1).start(priority=LP))

    def dma_mid(i, outs):
        dma_starts(i, False, outs)
        kv_copy(i, 2).wait()

    def unit_main(i):
        dma_top(i)
        kv_copy(i, 2).wait()
        when(i + SK == B, lambda: x_copy(3).wait())
        x_v[(i + SK) & 7] = xt_v[(i + SK) >> 3, (i + SK) & 7].T
        finish(jnp.maximum(i - 1, 0))

        def qh():
            when(i + SK == B, lambda: wqb_copy().wait())
            qproj(i + SK)
        attention(i, {Hkv - 1: qh})
        dma_starts(i, True, (i - 2,))
        when((i & 7) == 0,
             lambda: pltpu.make_async_copy(woa, wo_v.at[i >> 3], sems.at[S_WO + (i >> 3)]).wait())
        outT_v[i & 7, pl.ds(pl.multiple_of((i >> 3) * D, 64), D), :] = oproj_val(i)

    x_copy(0).start(priority=0)
    wqa_copy(0).start(priority=LP)
    x_copy(1).start(priority=LP)
    for c in range(1, len(WQCH)):
        wqa_copy(c).start(priority=LP)
    outT_v[:, pl.ds(D, 64), :] = jnp.zeros((B, 64, Sq), BF16)
    outT_v[0, pl.ds(0, D), :] = jnp.zeros((D, Sq), BF16)

    def pchunk(u0, nu, cols):
        x0 = jnp.concatenate([x_v[u] for u in range(u0, u0 + nu)], axis=0)
        q = (jnp.dot(x0, wq_v[0, :, cols], preferred_element_type=F32) * SCALE).astype(BF16)
        for t in range(nu):
            q_v[u0 + t, :, cols] = q[t * Sq:(t + 1) * Sq]

    x_copy(0).wait()
    x_v[0] = xt_v[0, 0].T
    x_v[1] = xt_v[0, 1].T
    wqa_copy(0).wait()
    pchunk(0, 2, pl.ds(WQOFF[0], WQCH[0]))
    x_copy(1).wait()
    x_v[2] = xt_v[0, 2].T
    x_v[3] = xt_v[0, 3].T
    pchunk(2, 2, pl.ds(WQOFF[0], WQCH[0]))
    x_copy(2).start(priority=LP)
    kv_start(0)
    wqa_copy(1).wait()
    pchunk(0, SK, pl.ds(WQOFF[1], WQCH[1]))
    wo_copy(0).start(priority=LP)
    kv_start(1)

    def pbody(c, _):
        pltpu.make_async_copy(wqa.at[:, pl.ds(1024, PW)], wq_v.at[0, :, pl.ds(1024, PW)],
                              sems.at[S_WQ + 2 + c]).wait()
        pchunk(0, SK, pl.ds(pl.multiple_of(1024 + c * PW, 512), PW))
        return 0
    jax.lax.fori_loop(0, 3072 // PW, pbody, 0)
    x_copy(2).wait()

    def main(b, _):
        unit_main(2 * b)
        unit_main(2 * b + 1)
        return 0
    jax.lax.fori_loop(0, (NU - SK) // 2, main, 0)

    T0 = NU - SK
    dma_top(T0)
    finish(T0 - 1)
    attention(T0, {HH: lambda: dma_mid(T0, (T0 - 2, T0 - 1))})

    def tail(i, _):
        dma_top(i)
        fin_direct(i - 1)
        attention(i, {HH: lambda: dma_mid(i, (i - 1,))})
        return 0
    jax.lax.fori_loop(T0 + 1, NU, tail, 0)

    b = B - 1

    def part(lo, hi, k):
        cols = pl.ds(lo, hi - lo)
        return pltpu.make_async_copy(out_v.at[b, :, cols], out_hbm.at[b, :, cols], sems.at[S_END + k])
    parts = [part(0, 512, 0)]
    parts[0].start()
    r0 = 0
    for k, nt in enumerate(ENDSPLIT):
        nr = 128 * nt - (64 if k == 0 else 0)
        r = jax.lax.dot_general(wo_v[1, pl.ds(r0, nr), :], o_v[(NU - 1) & 1], (((1,), (1,)), ((), ())),
                                preferred_element_type=F32).astype(BF16)
        if k == 0:
            r = jnp.concatenate([outT_v[b, pl.ds(512, 64), :], r], axis=0)
        lo = 512 if k == 0 else D + r0
        out_v[b, :, pl.ds(lo, 128 * nt)] = r.T
        parts.append(part(lo, lo + 128 * nt, k + 1))
        parts[-1].start()
        r0 += nr
    for u in range(B, NU - 1):
        out_copy(u).wait()
    for p in parts:
        p.wait()


@jax.jit
def pallas_concat_heads__gqa_block_cached__gqa_block_cached__near_ridge_kernel(
    A_x: jax.Array,
    A_k_cache: jax.Array,
    A_v_cache: jax.Array,
    A_wq: jax.Array,
    A_wo: jax.Array,
    B_x: jax.Array,
    B_k_cache: jax.Array,
    B_v_cache: jax.Array,
    B_wq: jax.Array,
    B_wo: jax.Array,
):
    hbm = pl.BlockSpec(memory_space=pltpu.HBM)
    return pl.pallas_call(
        _kernel,
        grid=(),
        in_specs=[hbm] * 10,
        out_specs=hbm,
        out_shape=jax.ShapeDtypeStruct((B, Sq, 2 * D), BF16),
        scratch_shapes=[
            pltpu.VMEM((2, B, D, Sq), BF16),
            pltpu.VMEM((8, Sq, D), BF16),
            pltpu.VMEM((2, D, HD), BF16),
            pltpu.VMEM((2, D, HD), BF16),
            pltpu.VMEM((NS, Hkv, Sk, Dh), BF16),
            pltpu.VMEM((NS, Hkv, Sk, Dh), BF16),
            pltpu.VMEM((8, Sq, HD), BF16),
            pltpu.VMEM((2, Sq, HD), BF16),
            pltpu.VMEM((B, 2 * D, Sq), BF16),
            pltpu.VMEM((B, Sq, 2 * D), BF16),
            pltpu.VMEM((2, 2 * Sq, Sk), BF16),
            pltpu.SemaphoreType.DMA((NSEM,)),
        ],
        compiler_params=pltpu.CompilerParams(
            vmem_limit_bytes=110 * 1024 * 1024,
            flags={"XLA_TPU_RESCHEDULE_DMA_DONES": True},
        ),
    )(A_x.transpose(0, 2, 1), A_k_cache, A_v_cache, A_wq, A_wo.T,
      B_x.transpose(0, 2, 1), B_k_cache, B_v_cache, B_wq, B_wo.T)
```
